```python
import jax
import jax.numpy as jnp

def _softmax(x, axis=-1):
    return jax.nn.softmax(x, axis=axis)
def _gelu(x):
    return jax.nn.gelu(x, approximate=True)
def _silu(x):
    return jax.nn.silu(x)
def _sigmoid(x):
    return jax.nn.sigmoid(x)
def _layernorm(x, axis=-1, eps=1e-5):
    m = jnp.mean(x, axis=axis, keepdims=True)
    v = jnp.var(x, axis=axis, keepdims=True)
    return (x - m) / jnp.sqrt(v + eps)
def _scatter_add(tgt, idx, src, axis=0):
    return tgt.at[idx].add(src)
def _segment_sum(src, seg, n):
    return jax.ops.segment_sum(src, seg, n)
class _Rng:
    def __init__(self, key):
        self._k = key
    def _next(self):
        self._k, sub = jax.random.split(self._k)
        return sub
    def normal(self, shape):
        return jax.random.normal(self._next(), shape, dtype=jnp.bfloat16)
    def randint(self, lo, hi, shape):
        return jax.random.randint(self._next(), shape, lo, hi, dtype=jnp.int32)
    def uniform(self, shape, lo=0.0, hi=1.0):
        return jax.random.uniform(self._next(), shape, jnp.bfloat16, lo, hi)
    def permutation(self, n):
        return jax.random.permutation(self._next(), n)


kernel_name = 'parallel_sum__gqa_block_cached__moe_arch_mod__decode'

def setup_inputs():
    _rng = _Rng(jax.random.key(int.from_bytes(__import__("os").urandom(4), "little")))
    _w = (lambda a: (lambda t: t.astype(jnp.bfloat16) if jnp.issubdtype(t.dtype, jnp.floating) else t)(jnp.asarray(a)))
    def _A_setup():
        B, Sq, D = 1, 1, 448
        Hq, Hkv, Sk, Dh = 16, 8, 65536, 256
        assert Hq % Hkv == 0, (Hq, Hkv)
        return {
            "x": _w((lambda *s: _rng.normal(s) * 0.05)(B, Sq, D)),
            "k_cache": _w((lambda *s: _rng.normal(s) * 0.05)(B, Hkv, Sk, Dh)),
            "v_cache": _w((lambda *s: _rng.normal(s) * 0.05)(B, Hkv, Sk, Dh)),
            "wq": _w((lambda *s: _rng.normal(s) * 0.05)(D, Hq * Dh) * (D ** -0.5)),
            "wo": _w((lambda *s: _rng.normal(s) * 0.05)(Hq * Dh, D) * ((Hq * Dh) ** -0.5)),
        }
    _A_in = _A_setup()

    def _B_setup():
        B, S, D, F, C = 1, 1, 448, 1792, 1
        return {
            "x": _w((lambda *s: _rng.normal(s) * 0.05)(B, S, D)),
            "w_r": _w((lambda *s: _rng.normal(s) * 0.05)(D)),
            "w_gate": _w((lambda *s: _rng.normal(s) * 0.05)(D, F)),
            "w_up": _w((lambda *s: _rng.normal(s) * 0.05)(D, F)),
            "w_down": _w((lambda *s: _rng.normal(s) * 0.05)(F, D)),
        }
    _B_in = _B_setup()

    return {
        "A_x": _A_in["x"],
        "A_k_cache": _A_in["k_cache"],
        "A_v_cache": _A_in["v_cache"],
        "A_wq": _A_in["wq"],
        "A_wo": _A_in["wo"],
        "B_x": _B_in["x"],
        "B_w_r": _B_in["w_r"],
        "B_w_gate": _B_in["w_gate"],
        "B_w_up": _B_in["w_up"],
        "B_w_down": _B_in["w_down"],
    }

def reference(A_x, A_k_cache, A_v_cache, A_wq, A_wo, B_x, B_w_r, B_w_gate, B_w_up, B_w_down):
    def _A_ref(x, k_cache, v_cache, wq, wo):
        B, Sq, D = x.shape
        Hq, Dh = 16, 256
        Hkv = k_cache.shape[1]
        rep = Hq // Hkv
        q = (lambda x, *d: x.transpose(*d))((x @ wq).reshape(B, Sq, Hq, Dh), 0, 2, 1, 3)
        k = jnp.repeat(k_cache, rep, axis=1)
        v = jnp.repeat(v_cache, rep, axis=1)
        scores = jnp.einsum("bhqd,bhkd->bhqk", q, k) * (Dh ** -0.5)
        p = _softmax(scores, axis=-1)
        o = jnp.einsum("bhqk,bhkd->bhqd", p, v)
        return (lambda x, *d: x.transpose(*d))(o, 0, 2, 1, 3).reshape(B, Sq, Hq * Dh) @ wo

    def _B_ref(x, w_r, w_gate, w_up, w_down):
        B, S, D = x.shape
        C = 1
        r = x @ w_r
        idx = jnp.argsort(-r, axis=-1)[:, :C]
        idx_e = jnp.repeat(idx.reshape(B, C, 1), D, axis=2)
        x_sel = jnp.take_along_axis(x, idx_e, axis=1)
        g = _silu(x_sel @ w_gate)
        u = x_sel @ w_up
        y = (g * u) @ w_down
        r_sel = _sigmoid(jnp.take_along_axis(r, idx, axis=1))
        y = y * r_sel.reshape(B, C, 1)
        b_off = (jnp.arange(B) * S).reshape(B, 1)
        flat_idx = (idx + b_off).reshape(B * C)
        zero = (x * 0.0).reshape(B * S, D)
        upd = _scatter_add(zero, flat_idx, y.reshape(B * C, D), axis=0)
        return x + upd.reshape(B, S, D)

    x = A_x
    xn = _layernorm(x, axis=-1)
    return x + _A_ref(xn, A_k_cache, A_v_cache, A_wq, A_wo) + _B_ref(xn, B_w_r, B_w_gate, B_w_up, B_w_down)
```

```python
import jax
import jax.numpy as jnp
from jax import lax
from jax.experimental import pallas as pl
from jax.experimental.pallas import tpu as pltpu

NT = (((1,), (1,)), ((), ()))
NN = (((1,), (0,)), ((), ()))

R = 1024
S = 8
NR = 32
NBUF = 4
PRIOS = (0, 1, 1, 0)
WPIECE = 256


def _kernel(x_ref, wr_ref, k_hbm, v_hbm, wq_hbm, wot_hbm, wg_hbm, wu_hbm, wdt_hbm,
            o_ref, kv, wq, wot, wg, wu, wdt, q_scr, kvsem, wsem, *, hkv, sk):
    d_model = x_ref.shape[-1]
    dh = k_hbm.shape[-1]
    nb = sk // R
    nsteps = hkv * nb
    seg = sk // S
    rs = R // S

    def start_step(t, slot):
        base = (t // nb) * sk + (t % nb) * rs
        c = 0
        for p in range(rs // NR):
            for s in range(S):
                for a, hbm in enumerate((k_hbm, v_hbm)):
                    src = hbm.at[pl.ds(pl.multiple_of(base + (s * seg + p * NR), NR), NR)]
                    dst = kv.at[slot, a, pl.ds(s * rs + p * NR, NR)]
                    pltpu.make_async_copy(src, dst, kvsem.at[slot]).start(
                        priority=PRIOS[c % len(PRIOS)])
                    c += 1

    def start_w(hbm, buf, idx):
        for p in range(hbm.shape[1] // WPIECE):
            cols = pl.ds(p * WPIECE, WPIECE)
            pltpu.make_async_copy(hbm.at[:, cols], buf.at[:, cols], wsem.at[idx]).start(
                priority=p % 2)

    def wait_w(buf, idx):
        pltpu.make_async_copy(buf, buf, wsem.at[idx]).wait()

    start_w(wq_hbm, wq, 0)
    for i in range(NBUF - 1):
        start_step(i, i)
        if i == 0:
            start_w(wg_hbm, wg, 1)
            start_w(wu_hbm, wu, 2)
            start_w(wdt_hbm, wdt, 3)
            start_w(wot_hbm, wot, 4)

    x = x_ref[0].astype(jnp.float32)
    xc = x - jnp.mean(x, axis=-1, keepdims=True)
    var = jnp.mean(xc * xc, axis=-1, keepdims=True)
    xn = xc / jnp.sqrt(var + 1e-5)
    xn8 = jnp.broadcast_to(xn.astype(jnp.bfloat16), (8, d_model))
    wait_w(wq, 0)
    q = lax.dot_general(xn8, wq[...], NN, preferred_element_type=jnp.float32)
    q = q * (dh ** -0.5)
    row = lax.broadcasted_iota(jnp.int32, (8, dh), 0)
    for hh in range(hkv):
        q_scr[hh] = jnp.where(row == 0, q[:, (2 * hh) * dh:(2 * hh + 1) * dh],
                              q[:, (2 * hh + 1) * dh:(2 * hh + 2) * dh])

    wait_w(wg, 1)
    g = lax.dot_general(xn8, wg[...], NN, preferred_element_type=jnp.float32)
    wait_w(wu, 2)
    u = lax.dot_general(xn8, wu[...], NN, preferred_element_type=jnp.float32)
    hid = (g * jax.nn.sigmoid(g)) * u
    wait_w(wdt, 3)
    y = lax.dot_general(hid.astype(jnp.bfloat16), wdt[...], NT,
                        preferred_element_type=jnp.float32)
    r = jnp.sum(xn * wr_ref[...].astype(jnp.float32).reshape(1, d_model), axis=-1, keepdims=True)
    y = y * jax.nn.sigmoid(r)
    rowd = lax.broadcasted_iota(jnp.int32, (8, d_model), 0)
    out0 = jnp.where(rowd == 0, jnp.broadcast_to(x + xn + y[0:1], (8, d_model)), 0.0)
    wait_w(wot, 4)

    def head_body(h, out):
        qh = q_scr[h].astype(jnp.bfloat16)

        def step(j, carry):
            m, l, acc = carry
            t = h * nb + j
            slot = t % NBUF

            @pl.when(t + NBUF - 1 < nsteps)
            def _():
                start_step(t + NBUF - 1, (t + NBUF - 1) % NBUF)

            pltpu.make_async_copy(kv.at[slot], kv.at[slot], kvsem.at[slot]).wait()
            s = lax.dot_general(qh, kv[slot, 0], NT, preferred_element_type=jnp.float32)
            m_new = jnp.maximum(m, jnp.max(s, axis=-1, keepdims=True))
            alpha = jnp.exp(m - m_new)
            p = jnp.exp(s - m_new)
            l = alpha * l + jnp.sum(p, axis=-1, keepdims=True)
            acc = alpha * acc + lax.dot_general(p.astype(jnp.bfloat16), kv[slot, 1], NN,
                                                preferred_element_type=jnp.float32)
            return m_new, l, acc

        _, l, acc = lax.fori_loop(0, nb, step, (jnp.full((8, 1), -jnp.inf, jnp.float32),
                                                jnp.zeros((8, 1), jnp.float32),
                                                jnp.zeros((8, dh), jnp.float32)))
        o = (acc / l).astype(jnp.bfloat16)
        off = pl.multiple_of(h * (2 * dh), 2 * dh)
        r0 = lax.dot_general(o, wot[:, pl.ds(off, dh)], NT, preferred_element_type=jnp.float32)
        r1 = lax.dot_general(o, wot[:, pl.ds(off + dh, dh)], NT, preferred_element_type=jnp.float32)
        return out + jnp.where(rowd == 0, r0, 0.0) + jnp.where(rowd == 1, r1, 0.0)

    out = lax.fori_loop(0, hkv, head_body, out0)
    o_ref[0] = jnp.sum(out, axis=0, keepdims=True).astype(o_ref.dtype)


@jax.jit
def pallas_parallel_sum__gqa_block_cached__moe_arch_mod__decode_kernel(
    A_x: jax.Array,
    A_k_cache: jax.Array,
    A_v_cache: jax.Array,
    A_wq: jax.Array,
    A_wo: jax.Array,
    B_x: jax.Array,
    B_w_r: jax.Array,
    B_w_gate: jax.Array,
    B_w_up: jax.Array,
    B_w_down: jax.Array,
):
    del B_x
    _, hkv, sk, dh = A_k_cache.shape
    d_model, f = B_w_gate.shape
    assert A_x.shape[:2] == (1, 1) and A_wq.shape[1] == 2 * hkv * dh
    assert sk % R == 0 and (R // S) % NR == 0
    assert A_wq.shape[1] % WPIECE == 0 and f % WPIECE == 0
    k = A_k_cache.reshape(hkv * sk, dh)
    v = A_v_cache.reshape(hkv * sk, dh)
    hbm = pl.BlockSpec(memory_space=pl.ANY)
    vmem = pl.BlockSpec(memory_space=pltpu.VMEM)
    bf16 = jnp.bfloat16
    kernel = lambda *refs: _kernel(*refs, hkv=hkv, sk=sk)
    return pl.pallas_call(
        kernel,
        in_specs=[vmem, vmem, hbm, hbm, hbm, hbm, hbm, hbm, hbm],
        out_specs=vmem,
        out_shape=jax.ShapeDtypeStruct(A_x.shape, A_x.dtype),
        scratch_shapes=[
            pltpu.VMEM((NBUF, 2, R, dh), bf16),
            pltpu.VMEM((d_model, 2 * hkv * dh), bf16),
            pltpu.VMEM((d_model, 2 * hkv * dh), bf16),
            pltpu.VMEM((d_model, f), bf16),
            pltpu.VMEM((d_model, f), bf16),
            pltpu.VMEM((d_model, f), bf16),
            pltpu.VMEM((hkv, 8, dh), jnp.float32),
            pltpu.SemaphoreType.DMA((NBUF,)),
            pltpu.SemaphoreType.DMA((5,)),
        ],
        compiler_params=pltpu.CompilerParams(vmem_limit_bytes=64 * 1024 * 1024),
    )(A_x, B_w_r, k, v, A_wq, A_wo.T, B_w_gate, B_w_up, B_w_down.T)
```

```python
import jax
import jax.numpy as jnp
from jax import lax
from jax.experimental import pallas as pl
from jax.experimental.pallas import tpu as pltpu

NT = (((1,), (1,)), ((), ()))
NN = (((1,), (0,)), ((), ()))

R = 1024
S = 8
NR = 32
NBUF = 4
PRIOS = (0, 1, 1, 0)
WPIECE = 256


def _kernel(x_hbm, wr_hbm, k_hbm, v_hbm, wq_hbm, wot_hbm, wg_hbm, wu_hbm, wdt_hbm,
            o_ref, kv, wq, wot, wg, wu, wdt, q_scr, x_ref, wr_ref, kvsem, wsem, *, hkv, sk):
    d_model = x_ref.shape[-1]
    dh = k_hbm.shape[-1]
    nb = sk // R
    nsteps = hkv * nb
    seg = sk // S
    rs = R // S

    def start_step(t, slot):
        base = (t // nb) * sk + (t % nb) * rs
        c = 0
        for p in range(rs // NR):
            for s in range(S):
                for a, hbm in enumerate((k_hbm, v_hbm)):
                    src = hbm.at[pl.ds(pl.multiple_of(base + (s * seg + p * NR), NR), NR)]
                    dst = kv.at[slot, a, pl.ds(s * rs + p * NR, NR)]
                    pltpu.make_async_copy(src, dst, kvsem.at[slot]).start(
                        priority=PRIOS[c % len(PRIOS)])
                    c += 1

    def start_w(hbm, buf, idx):
        for p in range(hbm.shape[1] // WPIECE):
            cols = pl.ds(p * WPIECE, WPIECE)
            pltpu.make_async_copy(hbm.at[:, cols], buf.at[:, cols], wsem.at[idx]).start(
                priority=p % 2)

    def wait_w(buf, idx):
        pltpu.make_async_copy(buf, buf, wsem.at[idx]).wait()

    cp_x = pltpu.make_async_copy(x_hbm, x_ref, wsem.at[5])
    cp_r = pltpu.make_async_copy(wr_hbm, wr_ref, wsem.at[6])
    cp_x.start()
    cp_r.start(priority=1)
    start_w(wq_hbm, wq, 0)
    for i in range(NBUF - 1):
        start_step(i, i)
        if i == 0:
            start_w(wg_hbm, wg, 1)
            start_w(wu_hbm, wu, 2)
            start_w(wdt_hbm, wdt, 3)
            start_w(wot_hbm, wot, 4)

    cp_x.wait()
    cp_r.wait()
    x = x_ref[0].astype(jnp.float32)
    xc = x - jnp.mean(x, axis=-1, keepdims=True)
    var = jnp.mean(xc * xc, axis=-1, keepdims=True)
    xn = xc / jnp.sqrt(var + 1e-5)
    xn8 = jnp.broadcast_to(xn.astype(jnp.bfloat16), (8, d_model))
    wait_w(wq, 0)
    q = lax.dot_general(xn8, wq[...], NN, preferred_element_type=jnp.float32)
    q = q * (dh ** -0.5)
    row = lax.broadcasted_iota(jnp.int32, (8, dh), 0)
    for hh in range(hkv):
        q_scr[hh] = jnp.where(row == 0, q[:, (2 * hh) * dh:(2 * hh + 1) * dh],
                              q[:, (2 * hh + 1) * dh:(2 * hh + 2) * dh])

    wait_w(wg, 1)
    g = lax.dot_general(xn8, wg[...], NN, preferred_element_type=jnp.float32)
    wait_w(wu, 2)
    u = lax.dot_general(xn8, wu[...], NN, preferred_element_type=jnp.float32)
    hid = (g * jax.nn.sigmoid(g)) * u
    wait_w(wdt, 3)
    y = lax.dot_general(hid.astype(jnp.bfloat16), wdt[...], NT,
                        preferred_element_type=jnp.float32)
    r = jnp.sum(xn * wr_ref[...].astype(jnp.float32).reshape(1, d_model), axis=-1, keepdims=True)
    y = y * jax.nn.sigmoid(r)
    rowd = lax.broadcasted_iota(jnp.int32, (8, d_model), 0)
    out0 = jnp.where(rowd == 0, jnp.broadcast_to(x + xn + y[0:1], (8, d_model)), 0.0)
    wait_w(wot, 4)

    def head_body(h, out):
        qh = q_scr[h].astype(jnp.bfloat16)

        def step(j, carry):
            m, l, acc = carry
            t = h * nb + j
            slot = t % NBUF

            @pl.when(t + NBUF - 1 < nsteps)
            def _():
                start_step(t + NBUF - 1, (t + NBUF - 1) % NBUF)

            pltpu.make_async_copy(kv.at[slot], kv.at[slot], kvsem.at[slot]).wait()
            s = lax.dot_general(qh, kv[slot, 0], NT, preferred_element_type=jnp.float32)
            m_new = jnp.maximum(m, jnp.max(s, axis=-1, keepdims=True))
            alpha = jnp.exp(m - m_new)
            p = jnp.exp(s - m_new)
            l = alpha * l + jnp.sum(p, axis=-1, keepdims=True)
            acc = alpha * acc + lax.dot_general(p.astype(jnp.bfloat16), kv[slot, 1], NN,
                                                preferred_element_type=jnp.float32)
            return m_new, l, acc

        _, l, acc = lax.fori_loop(0, nb, step, (jnp.full((8, 1), -jnp.inf, jnp.float32),
                                                jnp.zeros((8, 1), jnp.float32),
                                                jnp.zeros((8, dh), jnp.float32)))
        o = (acc / l).astype(jnp.bfloat16)
        off = pl.multiple_of(h * (2 * dh), 2 * dh)
        r0 = lax.dot_general(o, wot[:, pl.ds(off, dh)], NT, preferred_element_type=jnp.float32)
        r1 = lax.dot_general(o, wot[:, pl.ds(off + dh, dh)], NT, preferred_element_type=jnp.float32)
        return out + jnp.where(rowd == 0, r0, 0.0) + jnp.where(rowd == 1, r1, 0.0)

    out = lax.fori_loop(0, hkv, head_body, out0)
    o_ref[0] = jnp.sum(out, axis=0, keepdims=True).astype(o_ref.dtype)


@jax.jit
def pallas_parallel_sum__gqa_block_cached__moe_arch_mod__decode_kernel(
    A_x: jax.Array,
    A_k_cache: jax.Array,
    A_v_cache: jax.Array,
    A_wq: jax.Array,
    A_wo: jax.Array,
    B_x: jax.Array,
    B_w_r: jax.Array,
    B_w_gate: jax.Array,
    B_w_up: jax.Array,
    B_w_down: jax.Array,
):
    del B_x
    _, hkv, sk, dh = A_k_cache.shape
    d_model, f = B_w_gate.shape
    assert A_x.shape[:2] == (1, 1) and A_wq.shape[1] == 2 * hkv * dh
    assert sk % R == 0 and (R // S) % NR == 0
    assert A_wq.shape[1] % WPIECE == 0 and f % WPIECE == 0
    k = A_k_cache.reshape(hkv * sk, dh)
    v = A_v_cache.reshape(hkv * sk, dh)
    hbm = pl.BlockSpec(memory_space=pl.ANY)
    vmem = pl.BlockSpec(memory_space=pltpu.VMEM)
    bf16 = jnp.bfloat16
    kernel = lambda *refs: _kernel(*refs, hkv=hkv, sk=sk)
    return pl.pallas_call(
        kernel,
        in_specs=[hbm, hbm, hbm, hbm, hbm, hbm, hbm, hbm, hbm],
        out_specs=vmem,
        out_shape=jax.ShapeDtypeStruct(A_x.shape, A_x.dtype),
        scratch_shapes=[
            pltpu.VMEM((NBUF, 2, R, dh), bf16),
            pltpu.VMEM((d_model, 2 * hkv * dh), bf16),
            pltpu.VMEM((d_model, 2 * hkv * dh), bf16),
            pltpu.VMEM((d_model, f), bf16),
            pltpu.VMEM((d_model, f), bf16),
            pltpu.VMEM((d_model, f), bf16),
            pltpu.VMEM((hkv, 8, dh), jnp.float32),
            pltpu.VMEM(A_x.shape, A_x.dtype),
            pltpu.VMEM(B_w_r.shape, B_w_r.dtype),
            pltpu.SemaphoreType.DMA((NBUF,)),
            pltpu.SemaphoreType.DMA((7,)),
        ],
        compiler_params=pltpu.CompilerParams(vmem_limit_bytes=64 * 1024 * 1024),
    )(A_x, B_w_r, k, v, A_wq, A_wo.T, B_w_gate, B_w_up, B_w_down.T)
```
